```python
import os as _os
_os.environ.setdefault("JAX_PLATFORMS", "cpu")
import jax
import jax.numpy as jnp

def _softmax(x, axis=-1):
    return jax.nn.softmax(x, axis=axis)
def _gelu(x):
    return jax.nn.gelu(x, approximate=True)
def _silu(x):
    return jax.nn.silu(x)
def _sigmoid(x):
    return jax.nn.sigmoid(x)
def _layernorm(x, axis=-1, eps=1e-5):
    m = jnp.mean(x, axis=axis, keepdims=True)
    v = jnp.var(x, axis=axis, keepdims=True)
    return (x - m) / jnp.sqrt(v + eps)
def _scatter_add(tgt, idx, src, axis=0):
    return tgt.at[idx].add(src)
def _segment_sum(src, seg, n):
    return jax.ops.segment_sum(src, seg, n)
class _Rng:
    def __init__(self, key):
        self._k = key
    def _next(self):
        self._k, sub = jax.random.split(self._k)
        return sub
    def normal(self, shape):
        return jax.random.normal(self._next(), shape, dtype=jnp.bfloat16)
    def randint(self, lo, hi, shape):
        return jax.random.randint(self._next(), shape, lo, hi, dtype=jnp.int32)
    def uniform(self, shape, lo=0.0, hi=1.0):
        return jax.random.uniform(self._next(), shape, jnp.bfloat16, lo, hi)
    def permutation(self, n):
        return jax.random.permutation(self._next(), n)


kernel_name = 'parallel_sum__grouped_kv_mqa__dense_activation_silu__prompt'

def setup_inputs():
    _rng = _Rng(jax.random.key(int.from_bytes(__import__("os").urandom(4), "little")))
    _w = (lambda a: (lambda t: t.astype(jnp.bfloat16) if jnp.issubdtype(t.dtype, jnp.floating) else t)(jnp.asarray(a)))
    def _A_setup():
        B, S, D, H = 1, 2048, 512, 32
        Dh = D // H
        return {
            "x": _w((lambda *s: _rng.normal(s) * 0.05)(B, S, D)),
            "wq": _w((lambda *s: _rng.normal(s) * 0.05)(D, H * Dh)),
            "wk": _w((lambda *s: _rng.normal(s) * 0.05)(D, Dh)),
            "wv": _w((lambda *s: _rng.normal(s) * 0.05)(D, Dh)),
            "wo": _w((lambda *s: _rng.normal(s) * 0.05)(H * Dh, D)),
        }
    _A_in = _A_setup()

    def _B_setup():
        B, S, D, F = 1, 2048, 512, 1376
        return {
            "x": _w((lambda *s: _rng.normal(s) * 0.05)(B, S, D)),
            "w1": _w((lambda *s: _rng.normal(s) * 0.05)(D, F) * (D ** -0.5)),
            "w2": _w((lambda *s: _rng.normal(s) * 0.05)(F, D) * (F ** -0.5)),
        }
    _B_in = _B_setup()

    return {
        "A_x": _A_in["x"],
        "A_wq": _A_in["wq"],
        "A_wk": _A_in["wk"],
        "A_wv": _A_in["wv"],
        "A_wo": _A_in["wo"],
        "B_x": _B_in["x"],
        "B_w1": _B_in["w1"],
        "B_w2": _B_in["w2"],
    }

def reference(A_x, A_wq, A_wk, A_wv, A_wo, B_x, B_w1, B_w2):
    def _A_ref(x, wq, wk, wv, wo):
        B, S, D = x.shape
        H = 32
        Dh = D // H
        q = (lambda x, *d: x.transpose(*d))((x @ wq).reshape(B, S, H, Dh), 0, 2, 1, 3)
        k = x @ wk
        v = x @ wv
        scores = jnp.einsum("bhqd,bkd->bhqk", q, k) * (Dh ** -0.5)
        p = _softmax(scores, axis=-1)
        o = jnp.einsum("bhqk,bkd->bhqd", p, v)
        return (lambda x, *d: x.transpose(*d))(o, 0, 2, 1, 3).reshape(B, S, H * Dh) @ wo

    def _B_ref(x, w1, w2):
        h = jnp.einsum("bsd,df->bsf", x, w1)
        h = _silu(h)
        out = jnp.einsum("bsf,fd->bsd", h, w2)
        return out

    x = A_x
    xn = _layernorm(x, axis=-1)
    return x + _A_ref(xn, A_wq, A_wk, A_wv, A_wo) + _B_ref(xn, B_w1, B_w2)
```

```python
import functools
import jax
import jax.numpy as jnp
import jax.experimental.pallas as pl
import jax.experimental.pallas.tpu as pltpu

S, D, H, DH, F = 2048, 512, 32, 16, 1376
LOG2E = 1.4426950408889634
f32 = jnp.float32
bf16 = jnp.bfloat16


def _make(TQ=512, CK=128, LAG=2, TA=2, TL=2, TM=2, HPB=4):
    NQ = S // TQ
    NC = S // CK
    NL = TQ // 128
    assert HPB % 2 == 0

    def kernel(x_ref, wqt_ref, wkp_ref, wvt_ref, wo_ref, w1_ref, w2_ref, o_ref,
               xn_ref, kp_ref, vt_ref, qt_ref, sa_ref, sb_ref, ot_ref):
        qi = pl.program_id(0)

        @pl.when(qi == 0)
        def _():
            for r in range(S // 256):
                rs = slice(r * 256, (r + 1) * 256)
                x = x_ref[rs, :].astype(f32)
                mu = jnp.mean(x, axis=-1, keepdims=True)
                xc = x - mu
                var = jnp.mean(xc * xc, axis=-1, keepdims=True)
                xn = (xc * jax.lax.rsqrt(var + 1e-5)).astype(bf16)
                xn_ref[rs, :] = xn
                kp_ref[rs, :] = jnp.dot(xn, wkp_ref[...], preferred_element_type=f32).astype(bf16)
                vt_ref[:, rs] = jax.lax.dot_general(
                    wvt_ref[...], xn, (((1,), (1,)), ((), ())), preferred_element_type=f32).astype(bf16)
            qt_ref[D:, :] = jnp.zeros((128, TQ), bf16)
            if LAG:
                sb_ref[(NC - LAG) * CK:, :] = jnp.zeros((LAG * CK, TQ), f32)

        q0 = pl.multiple_of(qi * TQ, TQ)
        xq = xn_ref[pl.ds(q0, TQ), :]
        qt = jax.lax.dot_general(wqt_ref[...], xq, (((1,), (1,)), ((), ())), preferred_element_type=f32)
        qt_ref[0:D, :] = (qt * (0.25 * LOG2E)).astype(bf16)

        def pass1_chunk(h, s_ref, c, m):
            ks = slice(c * CK, (c + 1) * CK)
            w = qt_ref[pl.ds(pl.multiple_of(h * DH, DH), 128), :]
            k = kp_ref[ks, :]
            s = jnp.dot(k, w, preferred_element_type=f32)
            s_ref[ks, :] = s
            cm = jnp.max(s.reshape(CK // 8, 8, TQ), axis=0)
            return cm if m is None else jnp.maximum(m, cm)

        def pass2_chunk(s_ref, c, m, l, acc):
            ks = slice(c * CK, (c + 1) * CK)
            p = jnp.exp2(s_ref[ks, :].reshape(CK // 8, 8, TQ) - m[None])
            lc = jnp.sum(p, axis=0)
            oc = jnp.dot(vt_ref[:, ks], p.reshape(CK, TQ).astype(bf16), preferred_element_type=f32)
            if l is None:
                return lc, oc
            return l + lc, acc + oc

        def finish(h, l, acc):
            lsum = jnp.sum(l, axis=0, keepdims=True)
            ot_ref[pl.ds(pl.multiple_of((h + 1) * DH, DH), DH), :] = (acc / lsum).astype(bf16)

        def fin_max(m):
            return jnp.broadcast_to(jnp.max(m, axis=0, keepdims=True), (8, TQ))

        m = None
        for c in range(NC):
            m = pass1_chunk(0, sa_ref, c, m)
        m0 = fin_max(m)
        bufs = [sa_ref, sb_ref]

        def body(i, carry):
            m_prev, l_prev, acc_prev, m_cur = carry
            h0 = HPB * i
            mfin = {-1: m_prev, 0: m_cur}
            st = {-1: (l_prev, acc_prev)}
            mpart = None
            mhist = {}
            lhist = {}
            ahist = {}
            for s in range(HPB * NC):
                j1 = 1 + s // NC
                c1 = s % NC
                hp = jnp.minimum(h0 + j1, H - 1)
                mpart = pass1_chunk(hp, bufs[j1 % 2], c1, None if c1 == 0 else mpart)
                mhist[s] = mpart
                if c1 == NC - 1:
                    mfin[j1] = fin_max(mpart)
                g = s - LAG
                j2 = g // NC
                c2 = g % NC
                l, acc = st.get(j2, (None, None))
                mm = mfin[j2]
                deps = []
                if TA and (s - TA) in ahist: deps.append(ahist[s - TA][0:8, :])
                if TL and (s - TL) in lhist: deps.append(lhist[s - TL])
                if TM and (s - TM) in mhist: deps.append(mhist[s - TM])
                if deps:
                    d = functools.reduce(jnp.add, deps)
                    mm = jnp.where(d != d, d, mm)
                l, acc = pass2_chunk(bufs[j2 % 2], c2, mm, l, acc)
                lhist[s] = l
                ahist[s] = acc
                st[j2] = (l, acc)
                if c2 == NC - 1:
                    finish(h0 + j2, l, acc)
            if LAG:
                l1, a1 = st[HPB - 1]
            else:
                l1, a1 = l_prev, acc_prev
            return mfin[HPB - 1], l1, a1, mfin[HPB]

        init = (jnp.zeros((8, TQ), f32), jnp.ones((8, TQ), f32), jnp.zeros((DH, TQ), f32), m0)
        m_prev, l, acc, _ = jax.lax.fori_loop(0, H // HPB, body, init)
        for c in range(NC - LAG, NC):
            l, acc = pass2_chunk(sb_ref, c, m_prev, l, acc)
        if LAG:
            finish(H - 1, l, acc)

        att = jax.lax.dot_general(ot_ref[DH:, :], wo_ref[...], (((0,), (0,)), ((), ())), preferred_element_type=f32)
        hh = jnp.dot(xq, w1_ref[...], preferred_element_type=f32)
        hh = (hh * jax.nn.sigmoid(hh)).astype(bf16)
        ffn = jnp.dot(hh, w2_ref[...], preferred_element_type=f32)
        o_ref[...] = (x_ref[pl.ds(q0, TQ), :].astype(f32) + att + ffn).astype(o_ref.dtype)

    def fn(A_x, A_wq, A_wk, A_wv, A_wo, B_x, B_w1, B_w2):
        x = A_x.reshape(S, D)
        wqt = A_wq.T
        wkp = jnp.pad(A_wk, ((0, 0), (0, 128 - DH)))
        wvt = A_wv.T
        full = lambda shape: pl.BlockSpec(shape, lambda i: (0,) * len(shape))
        out = pl.pallas_call(
            kernel,
            grid=(NQ,),
            in_specs=[full((S, D)), full((D, D)), full((D, 128)), full((DH, D)), full((D, D)),
                      full((D, F)), full((F, D))],
            out_specs=pl.BlockSpec((TQ, D), lambda i: (i, 0)),
            out_shape=jax.ShapeDtypeStruct((S, D), bf16),
            scratch_shapes=[
                pltpu.VMEM((S, D), bf16),
                pltpu.VMEM((S, 128), bf16),
                pltpu.VMEM((DH, S), bf16),
                pltpu.VMEM((D + 128, TQ), bf16),
                pltpu.VMEM((S, TQ), f32),
                pltpu.VMEM((S, TQ), f32),
                pltpu.VMEM((D + DH, TQ), bf16),
            ],
            compiler_params=pltpu.CompilerParams(
                dimension_semantics=("arbitrary",), vmem_limit_bytes=100 * 1024 * 1024),
        )(x, wqt, wkp, wvt, A_wo, B_w1, B_w2)
        return out.reshape(1, S, D)
    return fn


_impl = _make()


@jax.jit
def pallas_parallel_sum__grouped_kv_mqa__dense_activation_silu__prompt_kernel(
    A_x: jax.Array,
    A_wq: jax.Array,
    A_wk: jax.Array,
    A_wv: jax.Array,
    A_wo: jax.Array,
    B_x: jax.Array,
    B_w1: jax.Array,
    B_w2: jax.Array,
):
    return _impl(A_x, A_wq, A_wk, A_wv, A_wo, B_x, B_w1, B_w2)
```

```python
import functools

import jax
import jax.numpy as jnp
import jax.experimental.pallas as pl
import jax.experimental.pallas.tpu as pltpu

S, D, H, DH, F = 2048, 512, 32, 16, 1376
LOG2E = 1.4426950408889634
f32 = jnp.float32
bf16 = jnp.bfloat16
u32 = jnp.uint32
NT_DIMS = (((1,), (1,)), ((), ()))
TN_DIMS = (((0,), (0,)), ((), ()))

TQ = 512
HPB = 16
DIST = 10
VREL = 6
NCAR = 2
CPOS = (2, 9)
RB = 256
L_MIN = 2.0 ** -40
L_MAX = 2.0 ** 13

NQ = S // TQ
NT = S // 128
NL = TQ // 128
TT = HPB * NT
NR = S // RB


def _kernel(x_hbm, wq_hbm, wk_hbm, wv_hbm, wo_hbm, w1_hbm, w2_hbm, o_ref,
            x_ref, wq_ref, wo_ref, w1_ref, w2_ref, sems,
            wt_ref, xn_ref, kp_ref, vt_ref, qa_ref, qf_ref, kt_ref, sq_ref, base_ref, kb_ref,
            pc_ref, au_ref, lu_ref, *qs_refs):
    qi = pl.program_id(0)

    def xcopy(r):
        return pltpu.make_async_copy(x_hbm.at[pl.ds(r * RB, RB)], x_ref.at[pl.ds(r * RB, RB)], sems.at[r])

    wcopies = [pltpu.make_async_copy(src, dst, sems.at[NR + n]) for n, (src, dst) in enumerate(
        [(wq_hbm, wq_ref), (wk_hbm, wt_ref.at[pl.ds(D, DH)]), (wv_hbm, wt_ref.at[pl.ds(D + DH, DH)]),
         (wo_hbm, wo_ref), (w1_hbm, w1_ref), (w2_hbm, w2_ref)])]

    @pl.when(qi == 0)
    def _():
        xcopy(0).start()
        for c in wcopies[:3]:
            c.start()
        for r in range(1, NR):
            xcopy(r).start()
        kns = []

        def ln(r):
            rs = slice(r * RB, (r + 1) * RB)
            x = x_ref[rs, :].astype(f32)
            mu = jnp.mean(x, axis=-1, keepdims=True)
            xc = x - mu
            var = jnp.mean(xc * xc, axis=-1, keepdims=True)
            xn_ref[rs, :] = (xc * jax.lax.rsqrt(var + 1e-5)).astype(bf16)

        def kv(r):
            rs = slice(r * RB, (r + 1) * RB)
            pt = jax.lax.dot_general(wt_ref[D:D + 2 * DH, :], xn_ref[rs, :], NT_DIMS, preferred_element_type=f32)
            kt = pt[0:DH, :].astype(bf16).astype(f32)
            kns.append(jnp.sum(kt * kt, axis=0, keepdims=True))
            kt_ref[:, rs] = kt
            vt_ref[:, rs] = pltpu.bitcast(pt[DH:2 * DH, :].astype(bf16), u32)

        def kpost(r):
            rs = slice(r * RB, (r + 1) * RB)
            rowi = jax.lax.broadcasted_iota(jnp.int32, (128 - DH, RB), 0)
            ktp = jnp.concatenate([kt_ref[:, rs], jnp.where(rowi < 2, 1.0, 0.0)], axis=0)
            kf = ktp.T
            kp_ref[r * RB // 2:(r + 1) * RB // 2, :] = pltpu.bitcast(kf.astype(bf16), u32)
            for cc in range(RB // 128):
                t = r * (RB // 128) + cc
                kvv = kf[cc * 128: cc * 128 + 16, :]
                for d in range(DH):
                    kb_ref[d, t * 16:(t + 1) * 16, :] = jnp.broadcast_to(kvv[:, d:d + 1], (16, 128))

        sel = (jax.lax.broadcasted_iota(jnp.int32, (64, 128), 0) * 2 ==
               (jax.lax.broadcasted_iota(jnp.int32, (64, 128), 1) // DH) * DH).astype(bf16)

        def qp(r):
            rs = slice(r * RB, (r + 1) * RB)
            pt = jax.lax.dot_general(wt_ref[0:D, :], xn_ref[rs, :], NT_DIMS, preferred_element_type=f32)
            qt_i, c0 = (r * RB) // TQ, (r * RB) % TQ
            cs = slice(c0, c0 + RB)
            qb16 = (pt * (0.25 * LOG2E)).astype(bf16)
            qb = qb16.astype(f32)
            qa_ref[qt_i, :, 0:8, cs] = pltpu.bitcast(qb16, u32).reshape(H, 8, RB)
            qf_ref[qt_i * H:(qt_i + 1) * H, 0:DH, cs] = qb.reshape(H, DH, RB)
            sq_ref[:, rs] = pltpu.bitcast((qb * qb).astype(bf16), u32)

        def aug(r, km):
            rs = slice(r * RB, (r + 1) * RB)
            qt_i, c0 = (r * RB) // TQ, (r * RB) % TQ
            cs = slice(c0, c0 + RB)
            n2 = jnp.concatenate(
                [jnp.dot(sel, pltpu.bitcast(sq_ref[k * 64:(k + 1) * 64, rs], bf16), preferred_element_type=f32)
                 for k in range(D // 128)], axis=0)
            rt = pltpu.bitcast(jax.lax.shift_right_logical(pltpu.bitcast(n2, u32), jnp.uint32(1))
                               + jnp.uint32(0x1fc00000), f32).reshape(H, 8, RB)
            hi = jax.lax.shift_right_logical(pltpu.bitcast(rt * km, u32), jnp.uint32(16))
            qa_ref[qt_i, :, 8:16, cs] = hi
            qf_ref[qt_i * H:(qt_i + 1) * H, DH:DH + 8, cs] = pltpu.bitcast(
                jax.lax.shift_left(hi, jnp.uint32(16)), f32)

        xcopy(0).wait()
        ln(0)
        for c in wcopies[:3]:
            c.wait()
        xcopy(1).wait()
        wt_ref[0:D, :] = wq_ref[...].T
        ln(1)
        kv(0)
        kv(1)
        xcopy(2).wait()
        xcopy(3).wait()
        kpost(0)
        kpost(1)
        qp(0)
        ln(2)
        ln(3)
        kv(2)
        kv(3)
        for r in range(4, NR):
            xcopy(r).wait()
        for c in wcopies[3:]:
            c.start()
        kpost(2)
        qp(1)
        ln(4)
        kv(4)
        kpost(3)
        qp(2)
        ln(5)
        kv(5)
        kpost(4)
        qp(3)
        ln(6)
        ln(7)
        kv(6)
        kv(7)
        kn = functools.reduce(jnp.maximum, kns)
        km = jnp.sqrt(jnp.max(kn, axis=1, keepdims=True)) * (-1.02)
        todo_k = list(range(5, NR))
        todo_a = list(range(NR))
        for r in range(4, NR):
            qp(r)
            for _ in range(-(-len(todo_k) // (NR - r))):
                if todo_k:
                    kpost(todo_k.pop(0))
            for _ in range(-(-(len(todo_a) - 1) // (NR - r))):
                if todo_a and todo_a[0] < r:
                    aug(todo_a.pop(0), km)
        for r in todo_a:
            aug(r, km)

    q0 = pl.multiple_of(qi * TQ, TQ)
    pc_ref[...] = jnp.zeros(pc_ref.shape, u32)

    def vtile(t):
        return pltpu.bitcast(vt_ref[:, t * 128:(t + 1) * 128], bf16)

    def finish(h, l, acc):
        au_ref[h + 1] = acc
        lu_ref[h + 1] = l

    def carried_pv(c, acc):
        p = pltpu.bitcast(pc_ref[c], bf16)
        return acc + jnp.dot(vtile(NT - NCAR + c), p, preferred_element_type=f32)

    def body(i, carry):
        l_c, acc_c = carry

        @pl.when(i >= 0)
        def _():
            for j in range(HPB):
                qs_refs[j][...] = qf_ref[qi * H + i * HPB + j, 0:DH, :]

        stream = [(T, pos) for T in range(TT) for pos in range(7)]
        last_m = {T: 7 * T + 6 for T in range(TT)}
        total_m = len(stream)
        pv_after = {T: min(last_m[T] + DIST, total_m - 1) for T in range(TT - NCAR)}
        cuts = sorted(set(pv_after.values()) | {last_m[j * NT + NT - 1] for j in range(HPB)} | set(CPOS))
        sg, pb, lsum, accs, ws = {}, {}, {}, {}, {}
        st = {'acc_c': acc_c}

        def proc(T, pos, s):
            j = T // NT
            p = jnp.exp2(s)
            l = lsum.get(j)
            pp = p[0:8, :] if l is None else l + p[0:8, :]
            lsum[j] = pp + p[8:16, :]
            pb[(T, pos)] = p

        def qk(g0, g1):
            j = stream[g0][0] // NT
            if j not in ws:
                ws[j] = pltpu.bitcast(qa_ref[qi, i * HPB + j], bf16)
            rows = []
            for g in range(g0, g1 + 1):
                T, pos = stream[g]
                a = (T % NT) * 8 + (7 - pos)
                rows.append(kp_ref[a * 8:(a + 1) * 8, :])
            kk = pltpu.bitcast(jnp.concatenate(rows, axis=0), bf16)
            s = jnp.dot(kk[:, 0:32], ws[j], preferred_element_type=f32)
            for g in range(g0, g1 + 1):
                sg[g] = s[(g - g0) * 16:(g - g0 + 1) * 16, :]
                proc(stream[g][0], stream[g][1], sg[g])

        def vqk(T):
            j, t = T // NT, T % NT
            qs = qs_refs[j]
            rel = last_m[T] - VREL
            acc = []
            for jj in range(NL):
                m = jnp.broadcast_to(qf_ref[qi * H + i * HPB + j, DH:DH + 1, jj * 128:(jj + 1) * 128], (8, 128))
                if rel in sg:
                    d = sg[rel][0:8, jj * 128:(jj + 1) * 128]
                    m = jnp.where(d != d, d, m)
                acc.append([m, m])
            for d in range(DH):
                kb = [kb_ref[d, t * 16 + 8 * r: t * 16 + 8 * r + 8, :] for r in range(2)]
                for jj in range(NL):
                    q = jnp.broadcast_to(qs[d:d + 1, jj * 128:(jj + 1) * 128], (8, 128))
                    for r in range(2):
                        acc[jj][r] = acc[jj][r] + kb[r] * q
            proc(T, 7, jnp.concatenate([jnp.concatenate(a_, axis=0) for a_ in acc], axis=1))

        def ptile(T):
            vqk(T)
            return jnp.concatenate([pb.pop((T, 7 - a)) for a in range(8)], axis=0).astype(bf16)

        def pv(T):
            j, t = T // NT, T % NT
            oc = jnp.dot(vtile(t), ptile(T), preferred_element_type=f32)
            if t == 0:
                o = accs[j - 1] if j > 0 else st['acc_c']
                acc = jnp.where(o != o, o, oc)
            else:
                acc = accs[j] + oc
            accs[j] = acc
            if t == NT - 1:
                finish(i * HPB + j, lsum[j], acc)

        g0 = 0
        for c in cuts:
            qk(g0, c)
            g0 = c + 1
            for cc in range(NCAR):
                if CPOS[cc] == c:
                    st['acc_c'] = carried_pv(cc, st['acc_c'])
                    if cc == NCAR - 1:
                        finish(i * HPB - 1, l_c, st['acc_c'])
            for T in range(TT - NCAR):
                if pv_after[T] == c:
                    pv(T)
        for cc in range(NCAR):
            pc_ref[cc] = pltpu.bitcast(ptile(TT - NCAR + cc), u32)
        return lsum[HPB - 1], accs[HPB - 1]

    init = (jnp.ones((8, TQ), f32), jnp.zeros((DH, TQ), f32))
    l_f, acc_f = jax.lax.fori_loop(0, H // HPB, body, init)

    @pl.when(qi == 0)
    def _():
        for c in wcopies[3:]:
            c.wait()

    for cc in range(NCAR):
        acc_f = carried_pv(cc, acc_f)
    finish(H - 1, l_f, acc_f)

    xq = xn_ref[pl.ds(q0, TQ), :]
    hh = jax.lax.dot_general(xq, w1_ref[...], NT_DIMS, preferred_element_type=f32)
    hx = 0.5 * hh
    hh = (hx + hx * jnp.tanh(hx)).astype(bf16)
    base = x_ref[pl.ds(q0, TQ), :].astype(f32) + jnp.dot(hh, w2_ref[...], preferred_element_type=f32)
    base_ref[...] = base

    def project(b):
        ls = jnp.sum(lu_ref[1:], axis=1, keepdims=True)
        ot = (au_ref[1:] / ls).reshape(D, TQ).astype(bf16)
        att = jax.lax.dot_general(ot, wo_ref[...], TN_DIMS, preferred_element_type=f32)
        o_ref[...] = (b + att).astype(o_ref.dtype)
        return ls

    ls = project(base)
    good = jnp.where(jnp.logical_and(ls >= L_MIN, ls <= L_MAX), 1.0, 0.0)
    ok = jnp.min(good) > 0.5

    @pl.when(jnp.logical_not(ok))
    def _():
        ckf = 256

        def fb_head(h, c):
            w = pltpu.bitcast(qa_ref[qi, h, 0:8, :], bf16)

            def scores(kc):
                r0 = pl.multiple_of(kc * (ckf // 2), ckf // 2)
                kk = pltpu.bitcast(kp_ref[pl.ds(r0, ckf // 2), :], bf16)
                return jnp.dot(kk[:, 0:DH], w, preferred_element_type=f32)

            def p1(kc, m):
                return jnp.maximum(m, jnp.max(scores(kc), axis=0, keepdims=True))
            m = jax.lax.fori_loop(0, S // ckf, p1, jnp.full((1, TQ), -jnp.inf, f32))

            def p2(kc, la):
                l_, a_ = la
                p = jnp.exp2(scores(kc) - m)
                c0 = pl.multiple_of(kc * ckf, ckf)
                v = pltpu.bitcast(vt_ref[:, pl.ds(c0, ckf)], bf16)
                return (l_ + jnp.sum(p.reshape(ckf // 8, 8, TQ), axis=0),
                        a_ + jnp.dot(v, p.astype(bf16), preferred_element_type=f32))
            l_, a_ = jax.lax.fori_loop(0, S // ckf, p2, (jnp.zeros((8, TQ), f32), jnp.zeros((DH, TQ), f32)))
            finish(h, l_, a_)
            return c
        jax.lax.fori_loop(0, H, fb_head, 0)
        project(base_ref[...])


@jax.jit
def pallas_parallel_sum__grouped_kv_mqa__dense_activation_silu__prompt_kernel(
    A_x: jax.Array,
    A_wq: jax.Array,
    A_wk: jax.Array,
    A_wv: jax.Array,
    A_wo: jax.Array,
    B_x: jax.Array,
    B_w1: jax.Array,
    B_w2: jax.Array,
):
    hbm = pl.BlockSpec(memory_space=pltpu.MemorySpace.HBM)
    out = pl.pallas_call(
        _kernel,
        grid=(NQ,),
        in_specs=[hbm] * 7,
        out_specs=pl.BlockSpec((TQ, D), lambda i: (i, 0)),
        out_shape=jax.ShapeDtypeStruct((S, D), bf16),
        scratch_shapes=[
            pltpu.VMEM((S, D), bf16),
            pltpu.VMEM((D, D), bf16),
            pltpu.VMEM((D, D), bf16),
            pltpu.VMEM((F, D), bf16),
            pltpu.VMEM((F, D), bf16),
            pltpu.SemaphoreType.DMA((NR + 6,)),
            pltpu.VMEM((D + 2 * DH, D), bf16),
            pltpu.VMEM((S, D), bf16),
            pltpu.VMEM((S // 2, 128), u32),
            pltpu.VMEM((DH // 2, S), u32),
            pltpu.VMEM((NQ, H, 16, TQ), u32),
            pltpu.VMEM((NQ * H, 24, TQ), f32),
            pltpu.VMEM((DH, S), f32),
            pltpu.VMEM((D // 2, S), u32),
            pltpu.VMEM((TQ, D), f32),
            pltpu.VMEM((DH, NT * 16, 128), f32),
            pltpu.VMEM((NCAR, 64, TQ), u32),
            pltpu.VMEM((H + 1, DH, TQ), f32),
            pltpu.VMEM((H + 1, 8, TQ), f32),
        ] + [pltpu.VMEM((DH, TQ), f32) for _ in range(HPB)],
        compiler_params=pltpu.CompilerParams(
            dimension_semantics=("arbitrary",), vmem_limit_bytes=100 * 1024 * 1024),
    )(A_x.reshape(S, D), A_wq, A_wk.T, A_wv.T, A_wo, B_w1.T, B_w2)
    return out.reshape(1, S, D)
```

```python
import functools

import jax
import jax.numpy as jnp
import jax.experimental.pallas as pl
import jax.experimental.pallas.tpu as pltpu

S, D, H, DH, F = 2048, 512, 32, 16, 1376
LOG2E = 1.4426950408889634
f32 = jnp.float32
bf16 = jnp.bfloat16
u32 = jnp.uint32
NT_DIMS = (((1,), (1,)), ((), ()))
TN_DIMS = (((0,), (0,)), ((), ()))

TQ = 512
HPB = 16
DIST = 10
VREL = 6
NCAR = 2
CPOS = (2, 9)
RB = 256
L_MIN = 2.0 ** -40
L_MAX = 2.0 ** 13

NQ = S // TQ
NT = S // 128
NL = TQ // 128
TT = HPB * NT
NR = S // RB
NI = H // HPB


def _kernel(x_hbm, wq_hbm, wk_hbm, wv_hbm, wo_hbm, w1_hbm, w2_hbm, o_ref,
            x_ref, wq_ref, wo_ref, w1_ref, w2_ref, sems,
            wt_ref, wkv_ref, xn_ref, kp_ref, vt_ref, qa_ref, qf_ref, mu_ref, mf_ref, kt_ref, sq_ref,
            base_ref, kb_ref, pc_ref, au_ref, lu_ref, *qs_refs):
    qi = pl.program_id(0)

    def xcopy(r):
        return pltpu.make_async_copy(x_hbm.at[pl.ds(r * RB, RB)], x_ref.at[pl.ds(r * RB, RB)], sems.at[r])

    wcopies = [pltpu.make_async_copy(src, dst, sems.at[NR + n]) for n, (src, dst) in enumerate(
        [(wq_hbm, wq_ref), (wk_hbm, wkv_ref.at[pl.ds(0, DH)]), (wv_hbm, wkv_ref.at[pl.ds(DH, DH)]),
         (wo_hbm, wo_ref), (w1_hbm, w1_ref), (w2_hbm, w2_ref)])]

    @pl.when(qi == 0)
    def _():
        xcopy(0).start()
        for c in wcopies[:3]:
            c.start()
        for r in range(1, NR):
            xcopy(r).start()
        kns = []

        def ln(r):
            rs = slice(r * RB, (r + 1) * RB)
            x = x_ref[rs, :].astype(f32)
            mu = jnp.mean(x, axis=-1, keepdims=True)
            xc = x - mu
            var = jnp.mean(xc * xc, axis=-1, keepdims=True)
            xn_ref[r * RB // 2:(r + 1) * RB // 2, :] = pltpu.bitcast(
                (xc * jax.lax.rsqrt(var + 1e-5)).astype(bf16), u32)

        def kv(r):
            rs = slice(r * RB, (r + 1) * RB)
            xb = pltpu.bitcast(xn_ref[r * RB // 2:(r + 1) * RB // 2, :], bf16)
            pt = jax.lax.dot_general(wkv_ref[...], xb, NT_DIMS, preferred_element_type=f32)
            kt = pt[0:DH, :].astype(bf16).astype(f32)
            kns.append(jnp.sum(kt * kt, axis=0, keepdims=True))
            kt_ref[:, rs] = kt
            vt_ref[:, rs] = pltpu.bitcast(pt[DH:2 * DH, :].astype(bf16), u32)

        def kpost(r):
            rs = slice(r * RB, (r + 1) * RB)
            rowi = jax.lax.broadcasted_iota(jnp.int32, (128 - DH, RB), 0)
            ktp = jnp.concatenate([kt_ref[:, rs], jnp.where(rowi < 2, 1.0, 0.0)], axis=0)
            kf = ktp.T
            kp_ref[r * RB // 2:(r + 1) * RB // 2, :] = pltpu.bitcast(kf.astype(bf16), u32)
            for cc in range(RB // 128):
                t = r * (RB // 128) + cc
                kvv = kf[cc * 128: cc * 128 + 16, :]
                for d in range(DH):
                    kb_ref[d, t * 16:(t + 1) * 16, :] = jnp.broadcast_to(kvv[:, d:d + 1], (16, 128))

        sel = (jax.lax.broadcasted_iota(jnp.int32, (16, 256), 0) ==
               jax.lax.broadcasted_iota(jnp.int32, (16, 256), 1) // DH).astype(bf16)

        def qh(c):
            rs = slice(c * 128, (c + 1) * 128)
            xb = pltpu.bitcast(xn_ref[c * 64:(c + 1) * 64, :], bf16)
            pt = jax.lax.dot_general(pltpu.bitcast(wt_ref[...], bf16), xb, NT_DIMS, preferred_element_type=f32)
            qt_i, c0 = (c * 128) // TQ, (c * 128) % TQ
            cs = slice(c0, c0 + 128)
            qb16 = (pt * (0.25 * LOG2E)).astype(bf16)
            qb = qb16.astype(f32)
            qa_ref[qt_i, :, :, cs] = pltpu.bitcast(qb16, u32).reshape(H, 8, 128)
            qf_ref[qt_i * H:(qt_i + 1) * H, :, cs] = qb.reshape(H, DH, 128)
            sq_ref[:, rs] = pltpu.bitcast((qb * qb).astype(bf16), u32)

        def aug(r, km):
            rs = slice(r * RB, (r + 1) * RB)
            qt_i, c0 = (r * RB) // TQ, (r * RB) % TQ
            cs = slice(c0, c0 + RB)
            n2 = jnp.concatenate(
                [jnp.dot(sel, pltpu.bitcast(sq_ref[k * 128:(k + 1) * 128, rs], bf16), preferred_element_type=f32)
                 for k in range(D // 256)], axis=0)
            rt = pltpu.bitcast(jax.lax.shift_right_logical(pltpu.bitcast(n2, u32), jnp.uint32(1))
                               + jnp.uint32(0x1fc00000), f32)
            hi = jax.lax.shift_right_logical(pltpu.bitcast(rt * km, u32), jnp.uint32(16))
            mu_ref[qt_i * NI:(qt_i + 1) * NI, :, cs] = hi.reshape(NI, HPB, RB)
            mf_ref[qt_i * NI:(qt_i + 1) * NI, :, cs] = pltpu.bitcast(
                jax.lax.shift_left(hi, jnp.uint32(16)), f32).reshape(NI, HPB, RB)

        xcopy(0).wait()
        ln(0)
        for c in wcopies[:3]:
            c.wait()
        xcopy(1).wait()
        wt_ref[...] = pltpu.bitcast(wq_ref[...].T, u32)
        kv(0); ln(1); kv(1); qh(0); qh(1)
        xcopy(2).wait()
        xcopy(3).wait()
        qh(2); ln(2); kv(2); qh(3); ln(3); kv(3)
        xcopy(4).wait()
        xcopy(5).wait()
        qh(4); ln(4); kv(4); qh(5); ln(5); kv(5)
        xcopy(6).wait()
        xcopy(7).wait()
        for c in wcopies[3:]:
            c.start()
        kpost(0)
        qh(6); ln(6); kv(6)
        kpost(1)
        qh(7); ln(7); kv(7)
        kn = functools.reduce(jnp.maximum, kns)
        km = jnp.sqrt(jnp.max(kn, axis=1, keepdims=True)) * (-1.02)
        for c in range(8, 16):
            if c - 6 < NR:
                kpost(c - 6)
            qh(c)
            if c >= 9:
                aug(c - 9, km)
        aug(7, km)

    q0 = pl.multiple_of(qi * TQ, TQ)
    pc_ref[...] = jnp.zeros(pc_ref.shape, u32)

    def vtile(t):
        return pltpu.bitcast(vt_ref[:, t * 128:(t + 1) * 128], bf16)

    def finish(h, l, acc):
        au_ref[h + 1] = acc
        lu_ref[h + 1] = l

    def carried_pv(c, acc):
        p = pltpu.bitcast(pc_ref[c], bf16)
        return acc + jnp.dot(vtile(NT - NCAR + c), p, preferred_element_type=f32)

    def body(i, carry):
        l_c, acc_c = carry

        @pl.when(i >= 0)
        def _():
            for j in range(HPB):
                qs_refs[j][...] = qf_ref[qi * H + i * HPB + j]

        stream = [(T, pos) for T in range(TT) for pos in range(7)]
        last_m = {T: 7 * T + 6 for T in range(TT)}
        total_m = len(stream)
        pv_after = {T: min(last_m[T] + DIST, total_m - 1) for T in range(TT - NCAR)}
        cuts = sorted(set(pv_after.values()) | {last_m[j * NT + NT - 1] for j in range(HPB)} | set(CPOS))
        sg, pb, lsum, accs, ws = {}, {}, {}, {}, {}
        st = {'acc_c': acc_c}

        def proc(T, pos, s):
            j = T // NT
            p = jnp.exp2(s)
            l = lsum.get(j)
            pp = p[0:8, :] if l is None else l + p[0:8, :]
            lsum[j] = pp + p[8:16, :]
            pb[(T, pos)] = p

        def qk(g0, g1):
            j = stream[g0][0] // NT
            if j not in ws:
                mrow = jnp.broadcast_to(mu_ref[qi * NI + i, j:j + 1, :], (8, TQ))
                ws[j] = pltpu.bitcast(jnp.concatenate([qa_ref[qi, i * HPB + j], mrow], axis=0), bf16)
            rows = []
            for g in range(g0, g1 + 1):
                T, pos = stream[g]
                a = (T % NT) * 8 + (7 - pos)
                rows.append(kp_ref[a * 8:(a + 1) * 8, :])
            kk = pltpu.bitcast(jnp.concatenate(rows, axis=0), bf16)
            s = jnp.dot(kk[:, 0:32], ws[j], preferred_element_type=f32)
            for g in range(g0, g1 + 1):
                sg[g] = s[(g - g0) * 16:(g - g0 + 1) * 16, :]
                proc(stream[g][0], stream[g][1], sg[g])

        def vqk(T):
            j, t = T // NT, T % NT
            qs = qs_refs[j]
            rel = last_m[T] - VREL
            acc = []
            for jj in range(NL):
                m = jnp.broadcast_to(mf_ref[qi * NI + i, j:j + 1, jj * 128:(jj + 1) * 128], (8, 128))
                if rel in sg:
                    d = sg[rel][0:8, jj * 128:(jj + 1) * 128]
                    m = jnp.where(d != d, d, m)
                acc.append([m, m])
            for d in range(DH):
                kb = [kb_ref[d, t * 16 + 8 * r: t * 16 + 8 * r + 8, :] for r in range(2)]
                for jj in range(NL):
                    q = jnp.broadcast_to(qs[d:d + 1, jj * 128:(jj + 1) * 128], (8, 128))
                    for r in range(2):
                        acc[jj][r] = acc[jj][r] + kb[r] * q
            proc(T, 7, jnp.concatenate([jnp.concatenate(a_, axis=0) for a_ in acc], axis=1))

        def ptile(T):
            vqk(T)
            return jnp.concatenate([pb.pop((T, 7 - a)) for a in range(8)], axis=0).astype(bf16)

        def pv(T):
            j, t = T // NT, T % NT
            oc = jnp.dot(vtile(t), ptile(T), preferred_element_type=f32)
            if t == 0:
                o = accs[j - 1] if j > 0 else st['acc_c']
                acc = jnp.where(o != o, o, oc)
            else:
                acc = accs[j] + oc
            accs[j] = acc
            if t == NT - 1:
                finish(i * HPB + j, lsum[j], acc)

        g0 = 0
        for c in cuts:
            qk(g0, c)
            g0 = c + 1
            for cc in range(NCAR):
                if CPOS[cc] == c:
                    st['acc_c'] = carried_pv(cc, st['acc_c'])
                    if cc == NCAR - 1:
                        finish(i * HPB - 1, l_c, st['acc_c'])
            for T in range(TT - NCAR):
                if pv_after[T] == c:
                    pv(T)
        for cc in range(NCAR):
            pc_ref[cc] = pltpu.bitcast(ptile(TT - NCAR + cc), u32)
        return lsum[HPB - 1], accs[HPB - 1]

    init = (jnp.ones((8, TQ), f32), jnp.zeros((DH, TQ), f32))
    l_f, acc_f = jax.lax.fori_loop(0, NI, body, init)

    @pl.when(qi == 0)
    def _():
        for c in wcopies[3:]:
            c.wait()

    for cc in range(NCAR):
        acc_f = carried_pv(cc, acc_f)
    finish(H - 1, l_f, acc_f)

    xq = pltpu.bitcast(xn_ref[pl.ds(pl.multiple_of(qi * (TQ // 2), TQ // 2), TQ // 2), :], bf16)
    hh = jax.lax.dot_general(xq, w1_ref[...], NT_DIMS, preferred_element_type=f32)
    hx = 0.5 * hh
    hh = (hx + hx * jnp.tanh(hx)).astype(bf16)
    base = x_ref[pl.ds(q0, TQ), :].astype(f32) + jnp.dot(hh, w2_ref[...], preferred_element_type=f32)
    base_ref[...] = base

    def project(b):
        ls = jnp.sum(lu_ref[1:], axis=1, keepdims=True)
        ot = (au_ref[1:] / ls).reshape(D, TQ).astype(bf16)
        att = jax.lax.dot_general(ot, wo_ref[...], TN_DIMS, preferred_element_type=f32)
        o_ref[...] = (b + att).astype(o_ref.dtype)
        return ls

    ls = project(base)
    good = jnp.where(jnp.logical_and(ls >= L_MIN, ls <= L_MAX), 1.0, 0.0)
    ok = jnp.min(good) > 0.5

    @pl.when(jnp.logical_not(ok))
    def _():
        ckf = 256

        def fb_head(h, c):
            w = pltpu.bitcast(qa_ref[qi, h], bf16)

            def scores(kc):
                r0 = pl.multiple_of(kc * (ckf // 2), ckf // 2)
                kk = pltpu.bitcast(kp_ref[pl.ds(r0, ckf // 2), :], bf16)
                return jnp.dot(kk[:, 0:DH], w, preferred_element_type=f32)

            def p1(kc, m):
                return jnp.maximum(m, jnp.max(scores(kc), axis=0, keepdims=True))
            m = jax.lax.fori_loop(0, S // ckf, p1, jnp.full((1, TQ), -jnp.inf, f32))

            def p2(kc, la):
                l_, a_ = la
                p = jnp.exp2(scores(kc) - m)
                c0 = pl.multiple_of(kc * ckf, ckf)
                v = pltpu.bitcast(vt_ref[:, pl.ds(c0, ckf)], bf16)
                return (l_ + jnp.sum(p.reshape(ckf // 8, 8, TQ), axis=0),
                        a_ + jnp.dot(v, p.astype(bf16), preferred_element_type=f32))
            l_, a_ = jax.lax.fori_loop(0, S // ckf, p2, (jnp.zeros((8, TQ), f32), jnp.zeros((DH, TQ), f32)))
            finish(h, l_, a_)
            return c
        jax.lax.fori_loop(0, H, fb_head, 0)
        project(base_ref[...])


@jax.jit
def pallas_parallel_sum__grouped_kv_mqa__dense_activation_silu__prompt_kernel(
    A_x: jax.Array,
    A_wq: jax.Array,
    A_wk: jax.Array,
    A_wv: jax.Array,
    A_wo: jax.Array,
    B_x: jax.Array,
    B_w1: jax.Array,
    B_w2: jax.Array,
):
    hbm = pl.BlockSpec(memory_space=pltpu.MemorySpace.HBM)
    out = pl.pallas_call(
        _kernel,
        grid=(NQ,),
        in_specs=[hbm] * 7,
        out_specs=pl.BlockSpec((TQ, D), lambda i: (i, 0)),
        out_shape=jax.ShapeDtypeStruct((S, D), bf16),
        scratch_shapes=[
            pltpu.VMEM((S, D), bf16),
            pltpu.VMEM((D, D), bf16),
            pltpu.VMEM((D, D), bf16),
            pltpu.VMEM((F, D), bf16),
            pltpu.VMEM((F, D), bf16),
            pltpu.SemaphoreType.DMA((NR + 6,)),
            pltpu.VMEM((D // 2, D), u32),
            pltpu.VMEM((2 * DH, D), bf16),
            pltpu.VMEM((S // 2, D), u32),
            pltpu.VMEM((S // 2, 128), u32),
            pltpu.VMEM((DH // 2, S), u32),
            pltpu.VMEM((NQ, H, 8, TQ), u32),
            pltpu.VMEM((NQ * H, DH, TQ), f32),
            pltpu.VMEM((NQ * NI, HPB, TQ), u32),
            pltpu.VMEM((NQ * NI, HPB, TQ), f32),
            pltpu.VMEM((DH, S), f32),
            pltpu.VMEM((D // 2, S), u32),
            pltpu.VMEM((TQ, D), f32),
            pltpu.VMEM((DH, NT * 16, 128), f32),
            pltpu.VMEM((NCAR, 64, TQ), u32),
            pltpu.VMEM((H + 1, DH, TQ), f32),
            pltpu.VMEM((H + 1, 8, TQ), f32),
        ] + [pltpu.VMEM((DH, TQ), f32) for _ in range(HPB)],
        compiler_params=pltpu.CompilerParams(
            dimension_semantics=("arbitrary",), vmem_limit_bytes=100 * 1024 * 1024),
    )(A_x.reshape(S, D), A_wq, A_wk.T, A_wv.T, A_wo, B_w1.T, B_w2)
    return out.reshape(1, S, D)
```

```python
import bisect
import functools

import jax
import jax.numpy as jnp
import jax.experimental.pallas as pl
import jax.experimental.pallas.tpu as pltpu

S, D, H, DH, F = 2048, 512, 32, 16, 1376
LOG2E = 1.4426950408889634
f32 = jnp.float32
bf16 = jnp.bfloat16
u32 = jnp.uint32
NT_DIMS = (((1,), (1,)), ((), ()))
TN_DIMS = (((0,), (0,)), ((), ()))
NANBITS = 0x7fc07fc0

TQ = 512
HPB = 16
DIST = 10
LEAD = 15.0
DMIN = 2.0
NCAR = 2
CPOS = (2, 9)
JS = (1, 5, 9, 13)
S0, GAP, TOKS, TST, PVLAG = 24, 10, 21, (0, 2, 4, 6), 8
RB = 256
FM = 128
L_MIN = 2.0 ** -40
L_MAX = 2.0 ** 13

NQ = S // TQ
NT = S // 128
NL = TQ // 128
NR = S // RB
NI = H // HPB
XH = [i * HPB + j for i in range(NI) for j in JS]
NXQ = len(XH) - len(JS)
FT = [(n * 128, min(128, F - n * 128)) for n in range((F + 127) // 128)]
KB = NT * 16 + 112


def _kbrow(t, a):
    return t * 16 if a == 0 else NT * 16 + (a - 1) * 16


def _silu(h):
    hx = 0.5 * h
    return hx + hx * jnp.tanh(hx)


def _kernel(x_hbm, wq_hbm, wk_hbm, wv_hbm, wo_hbm, w1_hbm, w2_hbm, o_ref,
            x_ref, wq_ref, wo_ref, w1_ref, w2_ref, sems,
            wt_ref, wkv_ref, xn_ref, kp_ref, vt_ref, qa_ref, qf_ref, mu_ref, mf_ref, kt_ref, sq_ref,
            base_ref, kb_ref, pc_ref, au_ref, lu_ref, hs_ref, qx_ref, *qs_refs):
    qi = pl.program_id(0)

    def xcopy(r):
        return pltpu.make_async_copy(x_hbm.at[pl.ds(r * RB, RB)], x_ref.at[pl.ds(r * RB, RB)], sems.at[r])

    wcopies = [pltpu.make_async_copy(src, dst, sems.at[NR + n]) for n, (src, dst) in enumerate(
        [(wq_hbm, wq_ref), (wk_hbm, wkv_ref.at[pl.ds(0, DH)]), (wv_hbm, wkv_ref.at[pl.ds(DH, DH)]),
         (wo_hbm, wo_ref), (w1_hbm, w1_ref), (w2_hbm, w2_ref)])]

    @pl.when(qi == 0)
    def _():
        xcopy(0).start()
        for c in wcopies[:3]:
            c.start()
        for r in range(1, NR):
            xcopy(r).start()
        kns = []

        def ln(r):
            rs = slice(r * RB, (r + 1) * RB)
            x = x_ref[rs, :].astype(f32)
            mu = jnp.mean(x, axis=-1, keepdims=True)
            xc = x - mu
            var = jnp.mean(xc * xc, axis=-1, keepdims=True)
            xn_ref[r * RB // 2:(r + 1) * RB // 2, :] = pltpu.bitcast(
                (xc * jax.lax.rsqrt(var + 1e-5)).astype(bf16), u32)

        def kv(r):
            rs = slice(r * RB, (r + 1) * RB)
            xb = pltpu.bitcast(xn_ref[r * RB // 2:(r + 1) * RB // 2, :], bf16)
            pt = jax.lax.dot_general(wkv_ref[...], xb, NT_DIMS, preferred_element_type=f32)
            kt = pt[0:DH, :].astype(bf16).astype(f32)
            kns.append(jnp.sum(kt * kt, axis=0, keepdims=True))
            kt_ref[:, rs] = kt
            vt_ref[:, rs] = pltpu.bitcast(pt[DH:2 * DH, :].astype(bf16), u32)

        def kpost(r):
            rs = slice(r * RB, (r + 1) * RB)
            rowi = jax.lax.broadcasted_iota(jnp.int32, (128 - DH, RB), 0)
            ktp = jnp.concatenate([kt_ref[:, rs], jnp.where(rowi < 2, 1.0, 0.0)], axis=0)
            kf = ktp.T
            kp_ref[r * RB // 2:(r + 1) * RB // 2, :] = pltpu.bitcast(kf.astype(bf16), u32)
            for cc in range(RB // 128):
                t = r * (RB // 128) + cc
                kvv = kf[cc * 128: cc * 128 + 16, :]
                for d in range(DH):
                    kb_ref[d, t * 16:(t + 1) * 16, :] = jnp.broadcast_to(kvv[:, d:d + 1], (16, 128))
            if r == 0:
                kvv = kf[16:128, :]
                for d in range(DH):
                    kb_ref[d, NT * 16:NT * 16 + 112, :] = jnp.broadcast_to(kvv[:, d:d + 1], (112, 128))

        sel = (jax.lax.broadcasted_iota(jnp.int32, (16, 256), 0) ==
               jax.lax.broadcasted_iota(jnp.int32, (16, 256), 1) // DH).astype(bf16)

        def qh(c):
            rs = slice(c * 128, (c + 1) * 128)
            xb = pltpu.bitcast(xn_ref[c * 64:(c + 1) * 64, :], bf16)
            pt = jax.lax.dot_general(pltpu.bitcast(wt_ref[...], bf16), xb, NT_DIMS, preferred_element_type=f32)
            qt_i, c0 = (c * 128) // TQ, (c * 128) % TQ
            cs = slice(c0, c0 + 128)
            qb16 = (pt * (0.25 * LOG2E)).astype(bf16)
            qb = qb16.astype(f32)
            qa_ref[qt_i, :, :, cs] = pltpu.bitcast(qb16, u32).reshape(H, 8, 128)
            qf_ref[qt_i * H:(qt_i + 1) * H, :, cs] = qb.reshape(H, DH, 128)
            sq_ref[:, rs] = pltpu.bitcast((qb * qb).astype(bf16), u32)

        def aug(r, km):
            rs = slice(r * RB, (r + 1) * RB)
            qt_i, c0 = (r * RB) // TQ, (r * RB) % TQ
            cs = slice(c0, c0 + RB)
            n2 = jnp.concatenate(
                [jnp.dot(sel, pltpu.bitcast(sq_ref[k * 128:(k + 1) * 128, rs], bf16), preferred_element_type=f32)
                 for k in range(D // 256)], axis=0)
            rt = pltpu.bitcast(jax.lax.shift_right_logical(pltpu.bitcast(n2, u32), jnp.uint32(1))
                               + jnp.uint32(0x1fc00000), f32)
            hi = jax.lax.shift_right_logical(pltpu.bitcast(rt * km, u32), jnp.uint32(16))
            mu_ref[qt_i * NI:(qt_i + 1) * NI, :, cs] = hi.reshape(NI, HPB, RB)
            mf_ref[qt_i * NI:(qt_i + 1) * NI, :, cs] = pltpu.bitcast(
                jax.lax.shift_left(hi, jnp.uint32(16)), f32).reshape(NI, HPB, RB)

        xcopy(0).wait()
        ln(0)
        for c in wcopies[:3]:
            c.wait()
        xcopy(1).wait()
        wt_ref[...] = pltpu.bitcast(wq_ref[...].T, u32)
        kv(0); ln(1); kv(1); qh(0); qh(1)
        xcopy(2).wait()
        xcopy(3).wait()
        qh(2); ln(2); kv(2); qh(3); ln(3); kv(3)
        xcopy(4).wait()
        xcopy(5).wait()
        qh(4); ln(4); kv(4); qh(5); ln(5); kv(5)
        xcopy(6).wait()
        xcopy(7).wait()
        for c in wcopies[3:]:
            c.start()
        kpost(0)
        qh(6); ln(6); kv(6)
        kpost(1)
        qh(7); ln(7); kv(7)
        kn = functools.reduce(jnp.maximum, kns)
        km = jnp.sqrt(jnp.max(kn, axis=1, keepdims=True)) * (-1.02)
        for c in range(8, 16):
            if c - 6 < NR:
                kpost(c - 6)
            qh(c)
            if c >= 9:
                aug(c - 9, km)
        aug(7, km)

    q0 = pl.multiple_of(qi * TQ, TQ)
    xoff = pl.multiple_of(qi * (TQ // 2), TQ // 2)
    pc_ref[...] = jnp.zeros(pc_ref.shape, u32)
    for e in range(NXQ):
        qx_ref[e] = qf_ref[qi * H + XH[e]]

    def vtile(t):
        return pltpu.bitcast(vt_ref[:, t * 128:(t + 1) * 128], bf16)

    def finish(h, l, acc):
        au_ref[h + 1] = acc
        lu_ref[h + 1] = l

    def carried_pv(c, acc):
        p = pltpu.bitcast(pc_ref[c], bf16)
        return acc + jnp.dot(vtile(NT - NCAR + c), p, preferred_element_type=f32)

    def vgroup(qs, mref, r0, tok):
        acc = []
        for jj in range(NL):
            m = jnp.broadcast_to(mref[:, jj * 128:(jj + 1) * 128], (8, 128))
            if tok is not None and tok[jj] is not None:
                d = tok[jj]
                m = jnp.where(d != d, d, m)
            acc.append([m, m])
        for d in range(DH):
            kb = [kb_ref[d, r0 + 8 * r: r0 + 8 * r + 8, :] for r in range(2)]
            for jj in range(NL):
                q = jnp.broadcast_to(qs[d:d + 1, jj * 128:(jj + 1) * 128], (8, 128))
                for r in range(2):
                    acc[jj][r] = acc[jj][r] + kb[r] * q
        return jnp.concatenate([jnp.concatenate(a_, axis=0) for a_ in acc], axis=1)

    def body(i, carry):
        l_c, acc_c = carry

        @pl.when(i >= 0)
        def _():
            for j in range(HPB):
                qs_refs[j][...] = qf_ref[qi * H + i * HPB + j]

        tiles = [(j, t) for j in range(HPB) for t in range(NT) if not (t == 0 and j in JS)]
        TT = len(tiles)
        stream = [(T, pos) for T in range(TT) for pos in range(7)]
        last_m = {T: 7 * T + 6 for T in range(TT)}
        total_m = len(stream)
        pv_at = {}
        for T in range(TT - NCAR):
            pv_at.setdefault(min(last_m[T] + DIST, total_m - 1), []).append(T)
        cuts = sorted(set(pv_at) | {last_m[T] for T in range(TT) if tiles[T][1] == NT - 1} | set(CPOS))
        tg, tpv = [], {}
        tm = 0
        for g in range(total_m):
            tg.append(tm)
            tm += 1 + (1 if g in CPOS else 0)
            for T in pv_at.get(g, ()):
                tpv[T] = tm
                tm += 1
        for T in range(TT - NCAR, TT):
            tpv[T] = tg[last_m[T]] + DIST + 2
        rel = {}
        nxt = 1e9
        for u in reversed([(T, jj) for T in range(TT) for jj in range(NL)]):
            nxt = min(tpv[u[0]] - LEAD, nxt - DMIN)
            rel[u] = nxt
        sg, pb, lsum, accs, ws = {}, {}, {}, {}, {}
        st = {'acc_c': acc_c}

        def token(T, jj):
            r_ = rel[(T, jj)]
            g = min(bisect.bisect_right(tg, r_) - 1, len(sg) - 1)
            if g < 0:
                return None
            half = 1 if (r_ - tg[g]) >= 0.5 else 0
            return sg[g][8 * half:8 * half + 8, jj * 128:(jj + 1) * 128]

        def proc(T, pos, s):
            j = tiles[T][0]
            p = jnp.exp2(s)
            l = lsum.get(j)
            pp = p[0:8, :] if l is None else l + p[0:8, :]
            lsum[j] = pp + p[8:16, :]
            pb[(T, pos)] = p

        def qk(g0, g1):
            j = tiles[stream[g0][0]][0]
            if j not in ws:
                mrow = jnp.broadcast_to(mu_ref[qi * NI + i, j:j + 1, :], (8, TQ))
                ws[j] = pltpu.bitcast(jnp.concatenate([qa_ref[qi, i * HPB + j], mrow], axis=0), bf16)
            rows = []
            for g in range(g0, g1 + 1):
                T, pos = stream[g]
                a = tiles[T][1] * 8 + (7 - pos)
                rows.append(kp_ref[a * 8:(a + 1) * 8, :])
            kk = pltpu.bitcast(jnp.concatenate(rows, axis=0), bf16)
            s = jnp.dot(kk[:, 0:32], ws[j], preferred_element_type=f32)
            for g in range(g0, g1 + 1):
                sg[g] = s[(g - g0) * 16:(g - g0 + 1) * 16, :]
                proc(stream[g][0], stream[g][1], sg[g])

        def ptile(T):
            j, t = tiles[T]
            tok = [token(T, jj) for jj in range(NL)]
            proc(T, 7, vgroup(qs_refs[j], mf_ref.at[qi * NI + i, j:j + 1], _kbrow(t, 0), tok))
            return jnp.concatenate([pb.pop((T, 7 - a)) for a in range(8)], axis=0).astype(bf16)

        def pv(T):
            j, t = tiles[T]
            oc = jnp.dot(vtile(t), ptile(T), preferred_element_type=f32)
            if j not in accs:
                o = accs[j - 1] if j > 0 else st['acc_c']
                acc = jnp.where(o != o, o, oc)
            else:
                acc = accs[j] + oc
            accs[j] = acc
            if t == NT - 1:
                finish(i * HPB + j, lsum[j], acc)

        g0 = 0
        for c in cuts:
            qk(g0, c)
            g0 = c + 1
            for cc in range(NCAR):
                if CPOS[cc] == c:
                    st['acc_c'] = carried_pv(cc, st['acc_c'])
                    if cc == NCAR - 1:
                        finish(i * HPB - 1, l_c, st['acc_c'])
            for T in pv_at.get(c, ()):
                pv(T)
        for cc in range(NCAR):
            pc_ref[cc] = pltpu.bitcast(ptile(TT - NCAR + cc), u32)
        return lsum[HPB - 1], accs[HPB - 1]

    init = (jnp.ones((8, TQ), f32), jnp.zeros((DH, TQ), f32))
    l_f, acc_f = jax.lax.fori_loop(0, NI, body, init)

    @pl.when(qi == 0)
    def _():
        for c in wcopies[3:]:
            c.wait()

    for cc in range(NCAR):
        acc_f = carried_pv(cc, acc_f)
    finish(H - 1, l_f, acc_f)

    NB = TQ // FM
    SL = FM // 16
    units = [('a', n, k, b) for n in range(len(FT)) for b in range(NB) for k in range(4)]
    units += [('b', n, k, b) for b in range(NB) for n in range(4) for k in range(len(FT))]
    rounds = [units[4 * r:4 * r + 4] for r in range(len(units) // 4)]
    NG = 8 * len(XH)
    dl = [int(S0 + GAP * u) for u in range(NG)]
    assert (dl[-1] + PVLAG) // SL < len(rounds)
    facc, rres, xp, xl = {}, {}, {}, {}
    for r, us in enumerate(rounds):
        ties = {}
        for u in range(NG):
            if dl[u] // SL == r:
                e, a = u // 8, 7 - u % 8
                h = XH[e]
                qs = qx_ref.at[e] if e < NXQ else qs_refs[h % HPB]
                tss = [min(dl[u] - TOKS + TST[jj], r * SL - 1) for jj in range(NL)]
                tk = None
                if all(ts >= 0 and len(rres.get(ts // SL, ())) == NL for ts in tss):
                    tk = [rres[ts // SL][jj][(ts % SL) * 16:(ts % SL) * 16 + 8, :] for jj, ts in enumerate(tss)]
                p = jnp.exp2(vgroup(qs, mf_ref.at[qi * NI + h // HPB, h % HPB:h % HPB + 1], _kbrow(0, a), tk))
                l = p[0:8, :] + p[8:16, :]
                xl[e] = l if e not in xl else xl[e] + l
                xp[(e, a)] = p
                ties[dl[u] % SL] = l
        for ui, (ph, n, k, b) in enumerate(us):
            if ph == 'a':
                lhs = xn_ref[pl.ds(xoff + b * (FM // 2), FM // 2), k * 128:(k + 1) * 128]
            else:
                lhs = hs_ref[b * (FM // 2):(b + 1) * (FM // 2), FT[k][0]:FT[k][0] + FT[k][1]]
            if ties:
                parts = []
                prev = 0
                for o in sorted(ties):
                    d = ties[o][:, ui * 128:ui * 128 + lhs.shape[1]]
                    if o * 8 > prev:
                        parts.append(lhs[prev:o * 8, :])
                    parts.append(jnp.where(d != d, jnp.uint32(NANBITS), lhs[o * 8:o * 8 + 8, :]))
                    prev = o * 8 + 8
                if prev < FM // 2:
                    parts.append(lhs[prev:, :])
                lhs = jnp.concatenate(parts, axis=0)
            lhs = pltpu.bitcast(lhs, bf16)
            if ph == 'a':
                f0, fn_ = FT[n]
                part = jax.lax.dot_general(lhs, w1_ref[f0:f0 + fn_, k * 128:(k + 1) * 128], NT_DIMS,
                                           preferred_element_type=f32)
                key = ('a', n, b)
                facc[key] = part if k == 0 else facc[key] + part
                if k == 3:
                    hs_ref[b * (FM // 2):(b + 1) * (FM // 2), f0:f0 + fn_] = pltpu.bitcast(
                        _silu(facc.pop(key)).astype(bf16), u32)
                if fn_ < 128:
                    part = None
            else:
                f0, fn_ = FT[k]
                part = jnp.dot(lhs, w2_ref[f0:f0 + fn_, n * 128:(n + 1) * 128], preferred_element_type=f32)
                key = ('b', n, b)
                facc[key] = part if k == 0 else facc[key] + part
                if k == len(FT) - 1:
                    xr = x_ref[pl.ds(q0 + b * FM, FM), n * 128:(n + 1) * 128]
                    base_ref[b * FM:(b + 1) * FM, n * 128:(n + 1) * 128] = xr.astype(f32) + facc.pop(key)
            if part is not None:
                rres.setdefault(r, []).append(part)
        for e in range(len(XH)):
            if (dl[8 * e + 7] + PVLAG) // SL == r:
                h = XH[e]
                p = jnp.concatenate([xp.pop((e, a)) for a in range(8)], axis=0).astype(bf16)
                au_ref[h + 1] = au_ref[h + 1] + jnp.dot(vtile(0), p, preferred_element_type=f32)
                lu_ref[h + 1] = lu_ref[h + 1] + xl.pop(e)

    def project():
        ls = jnp.sum(lu_ref[1:], axis=1, keepdims=True)
        ot = (au_ref[1:] / ls).reshape(D, TQ).astype(bf16)
        att = jax.lax.dot_general(ot, wo_ref[...], TN_DIMS, preferred_element_type=f32)
        o_ref[...] = (base_ref[...] + att).astype(o_ref.dtype)
        return ls

    ls = project()
    good = jnp.where(jnp.logical_and(ls >= L_MIN, ls <= L_MAX), 1.0, 0.0)
    ok = jnp.min(good) > 0.5

    @pl.when(jnp.logical_not(ok))
    def _():
        ckf = 256

        def fb_head(h, c):
            w = pltpu.bitcast(qa_ref[qi, h], bf16)

            def scores(kc):
                r0 = pl.multiple_of(kc * (ckf // 2), ckf // 2)
                kk = pltpu.bitcast(kp_ref[pl.ds(r0, ckf // 2), :], bf16)
                return jnp.dot(kk[:, 0:DH], w, preferred_element_type=f32)

            def p1(kc, m):
                return jnp.maximum(m, jnp.max(scores(kc), axis=0, keepdims=True))
            m = jax.lax.fori_loop(0, S // ckf, p1, jnp.full((1, TQ), -jnp.inf, f32))

            def p2(kc, la):
                l_, a_ = la
                p = jnp.exp2(scores(kc) - m)
                c0 = pl.multiple_of(kc * ckf, ckf)
                v = pltpu.bitcast(vt_ref[:, pl.ds(c0, ckf)], bf16)
                return (l_ + jnp.sum(p.reshape(ckf // 8, 8, TQ), axis=0),
                        a_ + jnp.dot(v, p.astype(bf16), preferred_element_type=f32))
            l_, a_ = jax.lax.fori_loop(0, S // ckf, p2, (jnp.zeros((8, TQ), f32), jnp.zeros((DH, TQ), f32)))
            finish(h, l_, a_)
            return c
        jax.lax.fori_loop(0, H, fb_head, 0)

        def fb_ffn(b, c):
            rb = 64
            xb = pltpu.bitcast(xn_ref[pl.ds(pl.multiple_of(xoff + b * (rb // 2), rb // 2), rb // 2), :], bf16)
            hh = _silu(jax.lax.dot_general(xb, w1_ref[...], NT_DIMS, preferred_element_type=f32)).astype(bf16)
            xr = x_ref[pl.ds(pl.multiple_of(q0 + b * rb, rb), rb), :].astype(f32)
            base_ref[pl.ds(pl.multiple_of(b * rb, rb), rb), :] = xr + jnp.dot(hh, w2_ref[...], preferred_element_type=f32)
            return c
        jax.lax.fori_loop(0, TQ // 64, fb_ffn, 0)
        project()


@jax.jit
def pallas_parallel_sum__grouped_kv_mqa__dense_activation_silu__prompt_kernel(
    A_x: jax.Array,
    A_wq: jax.Array,
    A_wk: jax.Array,
    A_wv: jax.Array,
    A_wo: jax.Array,
    B_x: jax.Array,
    B_w1: jax.Array,
    B_w2: jax.Array,
):
    hbm = pl.BlockSpec(memory_space=pltpu.MemorySpace.HBM)
    out = pl.pallas_call(
        _kernel,
        grid=(NQ,),
        in_specs=[hbm] * 7,
        out_specs=pl.BlockSpec((TQ, D), lambda i: (i, 0)),
        out_shape=jax.ShapeDtypeStruct((S, D), bf16),
        scratch_shapes=[
            pltpu.VMEM((S, D), bf16),
            pltpu.VMEM((D, D), bf16),
            pltpu.VMEM((D, D), bf16),
            pltpu.VMEM((F, D), bf16),
            pltpu.VMEM((F, D), bf16),
            pltpu.SemaphoreType.DMA((NR + 6,)),
            pltpu.VMEM((D // 2, D), u32),
            pltpu.VMEM((2 * DH, D), bf16),
            pltpu.VMEM((S // 2, D), u32),
            pltpu.VMEM((S // 2, 128), u32),
            pltpu.VMEM((DH // 2, S), u32),
            pltpu.VMEM((NQ, H, 8, TQ), u32),
            pltpu.VMEM((NQ * H, DH, TQ), f32),
            pltpu.VMEM((NQ * NI, HPB, TQ), u32),
            pltpu.VMEM((NQ * NI, HPB, TQ), f32),
            pltpu.VMEM((DH, S), f32),
            pltpu.VMEM((D // 2, S), u32),
            pltpu.VMEM((TQ, D), f32),
            pltpu.VMEM((DH, KB, 128), f32),
            pltpu.VMEM((NCAR, 64, TQ), u32),
            pltpu.VMEM((H + 1, DH, TQ), f32),
            pltpu.VMEM((H + 1, 8, TQ), f32),
            pltpu.VMEM((TQ // 2, F), u32),
            pltpu.VMEM((NXQ, DH, TQ), f32),
        ] + [pltpu.VMEM((DH, TQ), f32) for _ in range(HPB)],
        compiler_params=pltpu.CompilerParams(
            dimension_semantics=("arbitrary",), vmem_limit_bytes=100 * 1024 * 1024),
    )(A_x.reshape(S, D), A_wq, A_wk.T, A_wv.T, A_wo, B_w1.T, B_w2)
    return out.reshape(1, S, D)
```

```python
import bisect
import functools

import jax
import jax.numpy as jnp
import jax.experimental.pallas as pl
import jax.experimental.pallas.tpu as pltpu

S, D, H, DH, F = 2048, 512, 32, 16, 1376
LOG2E = 1.4426950408889634
f32 = jnp.float32
bf16 = jnp.bfloat16
u32 = jnp.uint32
NT_DIMS = (((1,), (1,)), ((), ()))
TN_DIMS = (((0,), (0,)), ((), ()))
NANBITS = 0x7fc07fc0

TQ = 512
HPB = 16
DIST = 10
LEAD = 15.0
DMIN = 2.0
NCAR = 2
CPOS = (2, 9)
JS = (1, 5, 9, 13)
S0, GAP, TOKS, TST, PVLAG = 24, 10, 21, (0, 2, 4, 6), 8
RB = 256
FM = 128
OFFS = 64.0
L_MIN = 2.0 ** -40
L_MAX = 2.0 ** 76
V_MAX = 2.0 ** 48

NQ = S // TQ
NT = S // 128
NL = TQ // 128
NR = S // RB
NI = H // HPB
XH = [i * HPB + j for i in range(NI) for j in JS]
NXQ = len(XH) - len(JS)
FT = [(n * 128, min(128, F - n * 128)) for n in range((F + 127) // 128)]
KB = NT * 16 + 112


def _kbrow(t, a):
    return t * 16 if a == 0 else NT * 16 + (a - 1) * 16


def _silu(h):
    hx = 0.5 * h
    return hx + hx * jnp.tanh(hx)


def _kernel(x_hbm, wq_hbm, wk_hbm, wv_hbm, wo_hbm, w1_hbm, w2_hbm, o_ref,
            x_ref, wq_ref, wo_ref, w1_ref, w2_ref, sems,
            wt_ref, wkv_ref, xn_ref, kp_ref, vt_ref, qa_ref, qf_ref, mu_ref, mf_ref, kt_ref, sq_ref,
            base_ref, kb_ref, pc_ref, au_ref, lu_ref, hs_ref, qx_ref, vok_ref, *qs_refs):
    qi = pl.program_id(0)

    def xcopy(r):
        return pltpu.make_async_copy(x_hbm.at[pl.ds(r * RB, RB)], x_ref.at[pl.ds(r * RB, RB)], sems.at[r])

    wcopies = [pltpu.make_async_copy(src, dst, sems.at[NR + n]) for n, (src, dst) in enumerate(
        [(wq_hbm, wq_ref), (wk_hbm, wkv_ref.at[pl.ds(0, DH)]), (wv_hbm, wkv_ref.at[pl.ds(DH, DH)]),
         (wo_hbm, wo_ref), (w1_hbm, w1_ref), (w2_hbm, w2_ref)])]

    @pl.when(qi == 0)
    def _():
        xcopy(0).start()
        for c in wcopies[:3]:
            c.start()
        for r in range(1, NR):
            xcopy(r).start()
        kns = []
        vms = []

        def ln(r):
            rs = slice(r * RB, (r + 1) * RB)
            x = x_ref[rs, :].astype(f32)
            mu = jnp.mean(x, axis=-1, keepdims=True)
            xc = x - mu
            var = jnp.mean(xc * xc, axis=-1, keepdims=True)
            xn_ref[r * RB // 2:(r + 1) * RB // 2, :] = pltpu.bitcast(
                (xc * jax.lax.rsqrt(var + 1e-5)).astype(bf16), u32)

        def kv(r):
            rs = slice(r * RB, (r + 1) * RB)
            xb = pltpu.bitcast(xn_ref[r * RB // 2:(r + 1) * RB // 2, :], bf16)
            pt = jax.lax.dot_general(wkv_ref[...], xb, NT_DIMS, preferred_element_type=f32)
            kt = pt[0:DH, :].astype(bf16).astype(f32)
            kns.append(jnp.sum(kt * kt, axis=0, keepdims=True))
            kt_ref[:, rs] = kt
            vms.append(jnp.where(jnp.abs(pt[DH:2 * DH, :]) <= V_MAX, 1.0, 0.0))
            vt_ref[:, rs] = pltpu.bitcast(pt[DH:2 * DH, :].astype(bf16), u32)

        def kpost(r):
            rs = slice(r * RB, (r + 1) * RB)
            rowi = jax.lax.broadcasted_iota(jnp.int32, (128 - DH, RB), 0)
            ktp = jnp.concatenate([kt_ref[:, rs], jnp.where(rowi < 2, 1.0, 0.0)], axis=0)
            kf = ktp.T
            kp_ref[r * RB // 2:(r + 1) * RB // 2, :] = pltpu.bitcast(kf.astype(bf16), u32)
            for cc in range(RB // 128):
                t = r * (RB // 128) + cc
                kvv = kf[cc * 128: cc * 128 + 16, :]
                for d in range(DH):
                    kb_ref[d, t * 16:(t + 1) * 16, :] = jnp.broadcast_to(kvv[:, d:d + 1], (16, 128))
            if r == 0:
                kvv = kf[16:128, :]
                for d in range(DH):
                    kb_ref[d, NT * 16:NT * 16 + 112, :] = jnp.broadcast_to(kvv[:, d:d + 1], (112, 128))

        sel = (jax.lax.broadcasted_iota(jnp.int32, (16, 256), 0) ==
               jax.lax.broadcasted_iota(jnp.int32, (16, 256), 1) // DH).astype(bf16)

        def qh(c):
            rs = slice(c * 128, (c + 1) * 128)
            xb = pltpu.bitcast(xn_ref[c * 64:(c + 1) * 64, :], bf16)
            pt = jax.lax.dot_general(pltpu.bitcast(wt_ref[...], bf16), xb, NT_DIMS, preferred_element_type=f32)
            qt_i, c0 = (c * 128) // TQ, (c * 128) % TQ
            cs = slice(c0, c0 + 128)
            qb16 = (pt * (0.25 * LOG2E)).astype(bf16)
            qb = qb16.astype(f32)
            qa_ref[qt_i, :, :, cs] = pltpu.bitcast(qb16, u32).reshape(H, 8, 128)
            qf_ref[qt_i * H:(qt_i + 1) * H, :, cs] = qb.reshape(H, DH, 128)
            sq_ref[:, rs] = pltpu.bitcast((qb * qb).astype(bf16), u32)

        def aug(r, km):
            rs = slice(r * RB, (r + 1) * RB)
            qt_i, c0 = (r * RB) // TQ, (r * RB) % TQ
            cs = slice(c0, c0 + RB)
            n2 = jnp.concatenate(
                [jnp.dot(sel, pltpu.bitcast(sq_ref[k * 128:(k + 1) * 128, rs], bf16), preferred_element_type=f32)
                 for k in range(D // 256)], axis=0)
            rt = pltpu.bitcast(jax.lax.shift_right_logical(pltpu.bitcast(n2, u32), jnp.uint32(1))
                               + jnp.uint32(0x1fc00000), f32)
            hi = jax.lax.shift_right_logical(pltpu.bitcast(rt * km + OFFS, u32), jnp.uint32(16))
            mu_ref[qt_i * NI:(qt_i + 1) * NI, :, cs] = hi.reshape(NI, HPB, RB)
            mf_ref[qt_i * NI:(qt_i + 1) * NI, :, cs] = pltpu.bitcast(
                jax.lax.shift_left(hi, jnp.uint32(16)), f32).reshape(NI, HPB, RB)

        xcopy(0).wait()
        ln(0)
        for c in wcopies[:3]:
            c.wait()
        xcopy(1).wait()
        wt_ref[...] = pltpu.bitcast(wq_ref[...].T, u32)
        kv(0); ln(1); kv(1); qh(0); qh(1)
        xcopy(2).wait()
        xcopy(3).wait()
        qh(2); ln(2); kv(2); qh(3); ln(3); kv(3)
        xcopy(4).wait()
        xcopy(5).wait()
        qh(4); ln(4); kv(4); qh(5); ln(5); kv(5)
        xcopy(6).wait()
        xcopy(7).wait()
        for c in wcopies[3:]:
            c.start()
        kpost(0)
        qh(6); ln(6); kv(6)
        kpost(1)
        qh(7); ln(7); kv(7)
        kn = functools.reduce(jnp.maximum, kns)
        vok_ref[...] = functools.reduce(jnp.minimum, vms)
        km = jnp.sqrt(jnp.max(kn, axis=1, keepdims=True)) * (-1.02)
        for c in range(8, 16):
            if c - 6 < NR:
                kpost(c - 6)
            qh(c)
            if c >= 9:
                aug(c - 9, km)
        aug(7, km)

    q0 = pl.multiple_of(qi * TQ, TQ)
    xoff = pl.multiple_of(qi * (TQ // 2), TQ // 2)
    pc_ref[...] = jnp.zeros(pc_ref.shape, u32)
    for e in range(NXQ):
        qx_ref[e] = qf_ref[qi * H + XH[e]]

    def vtile(t):
        return pltpu.bitcast(vt_ref[:, t * 128:(t + 1) * 128], bf16)

    def finish(h, l, acc):
        au_ref[h + 1] = acc
        lu_ref[h + 1] = l

    def carried_pv(c, acc):
        p = pltpu.bitcast(pc_ref[c], bf16)
        return acc + jnp.dot(vtile(NT - NCAR + c), p, preferred_element_type=f32)

    def vgroup(qs, mref, r0, tok):
        acc = []
        for jj in range(NL):
            m = jnp.broadcast_to(mref[:, jj * 128:(jj + 1) * 128], (8, 128))
            if tok is not None and tok[jj] is not None:
                d = tok[jj]
                m = jnp.where(d != d, d, m)
            acc.append([m, m])
        for d in range(DH):
            kb = [kb_ref[d, r0 + 8 * r: r0 + 8 * r + 8, :] for r in range(2)]
            for jj in range(NL):
                q = jnp.broadcast_to(qs[d:d + 1, jj * 128:(jj + 1) * 128], (8, 128))
                for r in range(2):
                    acc[jj][r] = acc[jj][r] + kb[r] * q
        return jnp.concatenate([jnp.concatenate(a_, axis=0) for a_ in acc], axis=1)

    def body(i, carry):
        l_c, acc_c = carry

        @pl.when(i >= 0)
        def _():
            for j in range(HPB):
                qs_refs[j][...] = qf_ref[qi * H + i * HPB + j]

        tiles = [(j, t) for j in range(HPB) for t in range(NT) if not (t == 0 and j in JS)]
        TT = len(tiles)
        stream = [(T, pos) for T in range(TT) for pos in range(7)]
        last_m = {T: 7 * T + 6 for T in range(TT)}
        total_m = len(stream)
        pv_at = {}
        for T in range(TT - NCAR):
            pv_at.setdefault(min(last_m[T] + DIST, total_m - 1), []).append(T)
        cuts = sorted(set(pv_at) | {last_m[T] for T in range(TT) if tiles[T][1] == NT - 1} | set(CPOS))
        tg, tpv = [], {}
        tm = 0
        for g in range(total_m):
            tg.append(tm)
            tm += 1 + (1 if g in CPOS else 0)
            for T in pv_at.get(g, ()):
                tpv[T] = tm
                tm += 1
        for T in range(TT - NCAR, TT):
            tpv[T] = tg[last_m[T]] + DIST + 2
        rel = {}
        nxt = 1e9
        for u in reversed([(T, jj) for T in range(TT) for jj in range(NL)]):
            nxt = min(tpv[u[0]] - LEAD, nxt - DMIN)
            rel[u] = nxt
        sg, pb, lsum, accs, ws = {}, {}, {}, {}, {}
        st = {'acc_c': acc_c}

        def token(T, jj):
            r_ = rel[(T, jj)]
            g = min(bisect.bisect_right(tg, r_) - 1, len(sg) - 1)
            if g < 0:
                return None
            half = 1 if (r_ - tg[g]) >= 0.5 else 0
            return sg[g][8 * half:8 * half + 8, jj * 128:(jj + 1) * 128]

        def proc(T, pos, s):
            j = tiles[T][0]
            p = jnp.exp2(s)
            l = lsum.get(j)
            pp = p[0:8, :] if l is None else l + p[0:8, :]
            lsum[j] = pp + p[8:16, :]
            pb[(T, pos)] = p

        def qk(g0, g1):
            j = tiles[stream[g0][0]][0]
            if j not in ws:
                mrow = jnp.broadcast_to(mu_ref[qi * NI + i, j:j + 1, :], (8, TQ))
                ws[j] = pltpu.bitcast(jnp.concatenate([qa_ref[qi, i * HPB + j], mrow], axis=0), bf16)
            rows = []
            for g in range(g0, g1 + 1):
                T, pos = stream[g]
                a = tiles[T][1] * 8 + (7 - pos)
                rows.append(kp_ref[a * 8:(a + 1) * 8, :])
            kk = pltpu.bitcast(jnp.concatenate(rows, axis=0), bf16)
            s = jnp.dot(kk[:, 0:32], ws[j], preferred_element_type=f32)
            for g in range(g0, g1 + 1):
                sg[g] = s[(g - g0) * 16:(g - g0 + 1) * 16, :]
                proc(stream[g][0], stream[g][1], sg[g])

        def ptile(T):
            j, t = tiles[T]
            tok = [token(T, jj) for jj in range(NL)]
            proc(T, 7, vgroup(qs_refs[j], mf_ref.at[qi * NI + i, j:j + 1], _kbrow(t, 0), tok))
            return jnp.concatenate([pb.pop((T, 7 - a)) for a in range(8)], axis=0).astype(bf16)

        def pv(T):
            j, t = tiles[T]
            oc = jnp.dot(vtile(t), ptile(T), preferred_element_type=f32)
            if j not in accs:
                o = accs[j - 1] if j > 0 else st['acc_c']
                acc = jnp.where(o != o, o, oc)
            else:
                acc = accs[j] + oc
            accs[j] = acc
            if t == NT - 1:
                finish(i * HPB + j, lsum[j], acc)

        g0 = 0
        for c in cuts:
            qk(g0, c)
            g0 = c + 1
            for cc in range(NCAR):
                if CPOS[cc] == c:
                    st['acc_c'] = carried_pv(cc, st['acc_c'])
                    if cc == NCAR - 1:
                        finish(i * HPB - 1, l_c, st['acc_c'])
            for T in pv_at.get(c, ()):
                pv(T)
        for cc in range(NCAR):
            pc_ref[cc] = pltpu.bitcast(ptile(TT - NCAR + cc), u32)
        return lsum[HPB - 1], accs[HPB - 1]

    init = (jnp.ones((8, TQ), f32), jnp.zeros((DH, TQ), f32))
    l_f, acc_f = jax.lax.fori_loop(0, NI, body, init)

    @pl.when(qi == 0)
    def _():
        for c in wcopies[3:]:
            c.wait()

    for cc in range(NCAR):
        acc_f = carried_pv(cc, acc_f)
    finish(H - 1, l_f, acc_f)

    NB = TQ // FM
    SL = FM // 16
    units = [('a', n, k, b) for n in range(len(FT)) for b in range(NB) for k in range(4)]
    units += [('b', n, k, b) for b in range(NB) for n in range(4) for k in range(len(FT))]
    rounds = [units[4 * r:4 * r + 4] for r in range(len(units) // 4)]
    NG = 8 * len(XH)
    dl = [int(S0 + GAP * u) for u in range(NG)]
    assert (dl[-1] + PVLAG) // SL < len(rounds)
    facc, rres, xp, xl = {}, {}, {}, {}
    for r, us in enumerate(rounds):
        ties = {}
        for u in range(NG):
            if dl[u] // SL == r:
                e, a = u // 8, 7 - u % 8
                h = XH[e]
                qs = qx_ref.at[e] if e < NXQ else qs_refs[h % HPB]
                tss = [min(dl[u] - TOKS + TST[jj], r * SL - 1) for jj in range(NL)]
                tk = None
                if all(ts >= 0 and len(rres.get(ts // SL, ())) == NL for ts in tss):
                    tk = [rres[ts // SL][jj][(ts % SL) * 16:(ts % SL) * 16 + 8, :] for jj, ts in enumerate(tss)]
                p = jnp.exp2(vgroup(qs, mf_ref.at[qi * NI + h // HPB, h % HPB:h % HPB + 1], _kbrow(0, a), tk))
                l = p[0:8, :] + p[8:16, :]
                xl[e] = l if e not in xl else xl[e] + l
                xp[(e, a)] = p
                ties[dl[u] % SL] = l
        for ui, (ph, n, k, b) in enumerate(us):
            if ph == 'a':
                lhs = xn_ref[pl.ds(xoff + b * (FM // 2), FM // 2), k * 128:(k + 1) * 128]
            else:
                lhs = hs_ref[b * (FM // 2):(b + 1) * (FM // 2), FT[k][0]:FT[k][0] + FT[k][1]]
            if ties:
                parts = []
                prev = 0
                for o in sorted(ties):
                    d = ties[o][:, ui * 128:ui * 128 + lhs.shape[1]]
                    if o * 8 > prev:
                        parts.append(lhs[prev:o * 8, :])
                    parts.append(jnp.where(d != d, jnp.uint32(NANBITS), lhs[o * 8:o * 8 + 8, :]))
                    prev = o * 8 + 8
                if prev < FM // 2:
                    parts.append(lhs[prev:, :])
                lhs = jnp.concatenate(parts, axis=0)
            lhs = pltpu.bitcast(lhs, bf16)
            if ph == 'a':
                f0, fn_ = FT[n]
                part = jax.lax.dot_general(lhs, w1_ref[f0:f0 + fn_, k * 128:(k + 1) * 128], NT_DIMS,
                                           preferred_element_type=f32)
                key = ('a', n, b)
                facc[key] = part if k == 0 else facc[key] + part
                if k == 3:
                    hs_ref[b * (FM // 2):(b + 1) * (FM // 2), f0:f0 + fn_] = pltpu.bitcast(
                        _silu(facc.pop(key)).astype(bf16), u32)
                if fn_ < 128:
                    part = None
            else:
                f0, fn_ = FT[k]
                part = jnp.dot(lhs, w2_ref[f0:f0 + fn_, n * 128:(n + 1) * 128], preferred_element_type=f32)
                key = ('b', n, b)
                facc[key] = part if k == 0 else facc[key] + part
                if k == len(FT) - 1:
                    xr = x_ref[pl.ds(q0 + b * FM, FM), n * 128:(n + 1) * 128]
                    base_ref[b * FM:(b + 1) * FM, n * 128:(n + 1) * 128] = xr.astype(f32) + facc.pop(key)
            if part is not None:
                rres.setdefault(r, []).append(part)
        for e in range(len(XH)):
            if (dl[8 * e + 7] + PVLAG) // SL == r:
                h = XH[e]
                p = jnp.concatenate([xp.pop((e, a)) for a in range(8)], axis=0).astype(bf16)
                au_ref[h + 1] = au_ref[h + 1] + jnp.dot(vtile(0), p, preferred_element_type=f32)
                lu_ref[h + 1] = lu_ref[h + 1] + xl.pop(e)

    def project():
        ls = jnp.sum(lu_ref[1:], axis=1, keepdims=True)
        ot = (au_ref[1:] / ls).reshape(D, TQ).astype(bf16)
        att = jax.lax.dot_general(ot, wo_ref[...], TN_DIMS, preferred_element_type=f32)
        o_ref[...] = (base_ref[...] + att).astype(o_ref.dtype)
        return ls

    ls = project()
    good = jnp.where(jnp.logical_and(ls >= L_MIN, ls <= L_MAX), 1.0, 0.0)
    ok = jnp.minimum(jnp.min(good), jnp.min(vok_ref[...])) > 0.5

    @pl.when(jnp.logical_not(ok))
    def _():
        ckf = 256

        def fb_head(h, c):
            w = pltpu.bitcast(qa_ref[qi, h], bf16)

            def scores(kc):
                r0 = pl.multiple_of(kc * (ckf // 2), ckf // 2)
                kk = pltpu.bitcast(kp_ref[pl.ds(r0, ckf // 2), :], bf16)
                return jnp.dot(kk[:, 0:DH], w, preferred_element_type=f32)

            def p1(kc, m):
                return jnp.maximum(m, jnp.max(scores(kc), axis=0, keepdims=True))
            m = jax.lax.fori_loop(0, S // ckf, p1, jnp.full((1, TQ), -jnp.inf, f32))

            def p2(kc, la):
                l_, a_ = la
                p = jnp.exp2(scores(kc) - m)
                c0 = pl.multiple_of(kc * ckf, ckf)
                v = pltpu.bitcast(vt_ref[:, pl.ds(c0, ckf)], bf16)
                return (l_ + jnp.sum(p.reshape(ckf // 8, 8, TQ), axis=0),
                        a_ + jnp.dot(v, p.astype(bf16), preferred_element_type=f32))
            l_, a_ = jax.lax.fori_loop(0, S // ckf, p2, (jnp.zeros((8, TQ), f32), jnp.zeros((DH, TQ), f32)))
            finish(h, l_, a_)
            return c
        jax.lax.fori_loop(0, H, fb_head, 0)

        def fb_ffn(b, c):
            rb = 64
            xb = pltpu.bitcast(xn_ref[pl.ds(pl.multiple_of(xoff + b * (rb // 2), rb // 2), rb // 2), :], bf16)
            hh = _silu(jax.lax.dot_general(xb, w1_ref[...], NT_DIMS, preferred_element_type=f32)).astype(bf16)
            xr = x_ref[pl.ds(pl.multiple_of(q0 + b * rb, rb), rb), :].astype(f32)
            base_ref[pl.ds(pl.multiple_of(b * rb, rb), rb), :] = xr + jnp.dot(hh, w2_ref[...], preferred_element_type=f32)
            return c
        jax.lax.fori_loop(0, TQ // 64, fb_ffn, 0)
        project()


@jax.jit
def pallas_parallel_sum__grouped_kv_mqa__dense_activation_silu__prompt_kernel(
    A_x: jax.Array,
    A_wq: jax.Array,
    A_wk: jax.Array,
    A_wv: jax.Array,
    A_wo: jax.Array,
    B_x: jax.Array,
    B_w1: jax.Array,
    B_w2: jax.Array,
):
    hbm = pl.BlockSpec(memory_space=pltpu.MemorySpace.HBM)
    out = pl.pallas_call(
        _kernel,
        grid=(NQ,),
        in_specs=[hbm] * 7,
        out_specs=pl.BlockSpec((TQ, D), lambda i: (i, 0)),
        out_shape=jax.ShapeDtypeStruct((S, D), bf16),
        scratch_shapes=[
            pltpu.VMEM((S, D), bf16),
            pltpu.VMEM((D, D), bf16),
            pltpu.VMEM((D, D), bf16),
            pltpu.VMEM((F, D), bf16),
            pltpu.VMEM((F, D), bf16),
            pltpu.SemaphoreType.DMA((NR + 6,)),
            pltpu.VMEM((D // 2, D), u32),
            pltpu.VMEM((2 * DH, D), bf16),
            pltpu.VMEM((S // 2, D), u32),
            pltpu.VMEM((S // 2, 128), u32),
            pltpu.VMEM((DH // 2, S), u32),
            pltpu.VMEM((NQ, H, 8, TQ), u32),
            pltpu.VMEM((NQ * H, DH, TQ), f32),
            pltpu.VMEM((NQ * NI, HPB, TQ), u32),
            pltpu.VMEM((NQ * NI, HPB, TQ), f32),
            pltpu.VMEM((DH, S), f32),
            pltpu.VMEM((D // 2, S), u32),
            pltpu.VMEM((TQ, D), f32),
            pltpu.VMEM((DH, KB, 128), f32),
            pltpu.VMEM((NCAR, 64, TQ), u32),
            pltpu.VMEM((H + 1, DH, TQ), f32),
            pltpu.VMEM((H + 1, 8, TQ), f32),
            pltpu.VMEM((TQ // 2, F), u32),
            pltpu.VMEM((NXQ, DH, TQ), f32),
            pltpu.VMEM((DH, RB), f32),
        ] + [pltpu.VMEM((DH, TQ), f32) for _ in range(HPB)],
        compiler_params=pltpu.CompilerParams(
            dimension_semantics=("arbitrary",), vmem_limit_bytes=100 * 1024 * 1024),
    )(A_x.reshape(S, D), A_wq, A_wk.T, A_wv.T, A_wo, B_w1.T, B_w2)
    return out.reshape(1, S, D)
```
